```python
import os as _os
_os.environ.setdefault("JAX_PLATFORMS", "cpu")
import jax
import jax.numpy as jnp

def _softmax(x, axis=-1):
    return jax.nn.softmax(x, axis=axis)
def _gelu(x):
    return jax.nn.gelu(x, approximate=True)
def _silu(x):
    return jax.nn.silu(x)
def _sigmoid(x):
    return jax.nn.sigmoid(x)
def _layernorm(x, axis=-1, eps=1e-5):
    m = jnp.mean(x, axis=axis, keepdims=True)
    v = jnp.var(x, axis=axis, keepdims=True)
    return (x - m) / jnp.sqrt(v + eps)
def _scatter_add(tgt, idx, src, axis=0):
    return tgt.at[idx].add(src)
def _segment_sum(src, seg, n):
    return jax.ops.segment_sum(src, seg, n)
class _Rng:
    def __init__(self, key):
        self._k = key
    def _next(self):
        self._k, sub = jax.random.split(self._k)
        return sub
    def normal(self, shape):
        return jax.random.normal(self._next(), shape, dtype=jnp.bfloat16)
    def randint(self, lo, hi, shape):
        return jax.random.randint(self._next(), shape, lo, hi, dtype=jnp.int32)
    def uniform(self, shape, lo=0.0, hi=1.0):
        return jax.random.uniform(self._next(), shape, jnp.bfloat16, lo, hi)
    def permutation(self, n):
        return jax.random.permutation(self._next(), n)


kernel_name = 'concat_heads__gqa_block_cached__mha_block_cached__near_ridge'

def setup_inputs():
    _rng = _Rng(jax.random.key(int.from_bytes(__import__("os").urandom(4), "little")))
    _w = (lambda a: (lambda t: t.astype(jnp.bfloat16) if jnp.issubdtype(t.dtype, jnp.floating) else t)(jnp.asarray(a)))
    def _A_setup():
        B, Sq, D = 16, 32, 1024
        Hq, Hkv, Sk, Dh = 32, 4, 32, 128
        assert Hq % Hkv == 0, (Hq, Hkv)
        return {
            "x": _w((lambda *s: _rng.normal(s) * 0.8)(B, Sq, D)),
            "k_cache": _w((lambda *s: _rng.normal(s) * 0.8)(B, Hkv, Sk, Dh)),
            "v_cache": _w((lambda *s: _rng.normal(s) * 0.05)(B, Hkv, Sk, Dh)),
            "wq": _w((lambda *s: _rng.normal(s) * 0.8)(D, Hq * Dh) * (D ** -0.5)),
            "wo": _w((lambda *s: _rng.normal(s) * 0.05)(Hq * Dh, D) * ((Hq * Dh) ** -0.5)),
        }
    _A_in = _A_setup()

    def _B_setup():
        B, Sq, D = 16, 32, 1024
        H, Sk, Dh = 32, 32, 128
        return {
            "x": _w((lambda *s: _rng.normal(s) * 0.8)(B, Sq, D)),
            "k_cache": _w((lambda *s: _rng.normal(s) * 0.8)(B, H, Sk, Dh)),
            "v_cache": _w((lambda *s: _rng.normal(s) * 0.05)(B, H, Sk, Dh)),
            "wq": _w((lambda *s: _rng.normal(s) * 0.8)(D, H * Dh) * (D ** -0.5)),
            "wo": _w((lambda *s: _rng.normal(s) * 0.05)(H * Dh, D) * ((H * Dh) ** -0.5)),
        }
    _B_in = _B_setup()

    return {
        "A_x": _A_in["x"],
        "A_k_cache": _A_in["k_cache"],
        "A_v_cache": _A_in["v_cache"],
        "A_wq": _A_in["wq"],
        "A_wo": _A_in["wo"],
        "B_x": _B_in["x"],
        "B_k_cache": _B_in["k_cache"],
        "B_v_cache": _B_in["v_cache"],
        "B_wq": _B_in["wq"],
        "B_wo": _B_in["wo"],
    }

def reference(A_x, A_k_cache, A_v_cache, A_wq, A_wo, B_x, B_k_cache, B_v_cache, B_wq, B_wo):
    def _A_ref(x, k_cache, v_cache, wq, wo):
        B, Sq, D = x.shape
        Hq, Dh = 32, 128
        Hkv = k_cache.shape[1]
        rep = Hq // Hkv
        q = (lambda x, *d: x.transpose(*d))((x @ wq).reshape(B, Sq, Hq, Dh), 0, 2, 1, 3)
        k = jnp.repeat(k_cache, rep, axis=1)
        v = jnp.repeat(v_cache, rep, axis=1)
        scores = jnp.einsum("bhqd,bhkd->bhqk", q, k) * (Dh ** -0.5)
        p = _softmax(scores, axis=-1)
        o = jnp.einsum("bhqk,bhkd->bhqd", p, v)
        return (lambda x, *d: x.transpose(*d))(o, 0, 2, 1, 3).reshape(B, Sq, Hq * Dh) @ wo

    def _B_ref(x, k_cache, v_cache, wq, wo):
        B, Sq, D = x.shape
        H, Dh = 32, 128
        q = (lambda x, *d: x.transpose(*d))((x @ wq).reshape(B, Sq, H, Dh), 0, 2, 1, 3)
        scores = jnp.einsum("bhqd,bhkd->bhqk", q, k_cache) * (Dh ** -0.5)
        p = _softmax(scores, axis=-1)
        o = jnp.einsum("bhqk,bhkd->bhqd", p, v_cache)
        return (lambda x, *d: x.transpose(*d))(o, 0, 2, 1, 3).reshape(B, Sq, H * Dh) @ wo

    a = _A_ref(A_x, A_k_cache, A_v_cache, A_wq, A_wo)
    b = _B_ref(B_x, B_k_cache, B_v_cache, B_wq, B_wo)
    return jnp.concatenate([a, b], axis=-1)
```

```python
import functools
import math
import jax
import jax.numpy as jnp
from jax import lax
import jax.experimental.pallas as pl
import jax.experimental.pallas.tpu as pltpu

B, SQ, D = 16, 32, 1024
H, DH, SK = 32, 128, 32
HKV = 4
M = B * SQ
HG = 4
NS = H // HG
CW = HG * DH
SCALE = DH ** -0.5
EXP2_SCALE = SCALE * math.log2(math.e)
F32 = jnp.float32
BF16 = jnp.bfloat16
U32 = jnp.uint32
KP = (128, 128, 256, 256, 256)
OUTC = (256, 256, 256, 128, 128)
WOP = D + 128
CONV = 80

_NT = (((1,), (1,)), ((), ()))


def _dot(a, b):
    return jnp.dot(a, b, preferred_element_type=F32)


def _dot_nt(a, b):
    return lax.dot_general(a, b, _NT, preferred_element_type=F32)


def _pack(x):
    return pltpu.bitcast(x.astype(BF16), U32)


def _unpack(x):
    return pltpu.bitcast(x, BF16)


def _softmax_t(st):
    m = jnp.max(st, axis=0, keepdims=True)
    e = jnp.exp2((st - m) * EXP2_SCALE)
    l = jnp.sum(e, axis=0, keepdims=True)
    r = pl.reciprocal(l, approx=True)
    r = r * (2.0 - l * r)
    return e * r


def kernel(xa_h, ka_h, va_h, wqa_h, woa_h, xb_h, kb_h, vb_h, wqb_h, wob_h, out_h,
           x_v, wq_v, wo_v, ka_v, va_v, kb_v, vb_v, q_v, pt_v, o_v, acc_v, outa_v, outb_v, sems):
    off = [0]

    def sem_block(n):
        r = sems.at[pl.ds(off[0], n)]
        off[0] += n
        return r

    sem_p = sem_block(len(KP))
    sem_s = sem_block(2 * NS)
    sem_out = sem_block(1)

    def cp_piece(i):
        k0 = sum(KP[:i])
        kk = pl.ds(k0, KP[i])
        return [
            pltpu.make_async_copy(xa_h.at[:, kk], x_v.at[0, :, kk], sem_p.at[i]),
            pltpu.make_async_copy(wqa_h.at[kk, pl.ds(0, CW)], wq_v.at[0, kk, :], sem_p.at[i]),
            pltpu.make_async_copy(wqa_h.at[kk, pl.ds(CW, CW)], wq_v.at[1, kk, :], sem_p.at[i]),
        ]

    def cp_xb(sem):
        return pltpu.make_async_copy(xb_h, x_v.at[1], sem)

    def cp_wq(s, sem):
        src = (wqa_h, wqb_h)[s // NS]
        c = s % NS
        return pltpu.make_async_copy(src.at[:, pl.ds(c * CW, CW)], wq_v.at[s], sem)

    def cp_wo(s, sem):
        src = (woa_h, wob_h)[s // NS]
        c = s % NS
        return pltpu.make_async_copy(src.at[pl.ds(c * CW, CW), :], wo_v.at[s, :, pl.ds(0, D)], sem)

    def cp_kva(part, sem):
        gs = pl.ds(0, 1) if part == 0 else pl.ds(1, HKV - 1)
        return [
            pltpu.make_async_copy(ka_h.at[:, gs], ka_v.at[:, gs], sem),
            pltpu.make_async_copy(va_h.at[:, gs], va_v.at[:, gs], sem),
        ]

    def cp_kvb(c, sem):
        return [
            pltpu.make_async_copy(kb_h.at[:, pl.ds(c * HG, HG)], kb_v.at[c], sem),
            pltpu.make_async_copy(vb_h.at[:, pl.ds(c * HG, HG)], vb_v.at[c], sem),
        ]

    def wait_wq(s, sem):
        pltpu.make_async_copy(wq_v.at[s], wq_v.at[s], sem).wait()

    def wait_wo(s, sem):
        r = wo_v.at[s, :, pl.ds(0, D)]
        pltpu.make_async_copy(r, r, sem).wait()

    def wait_kvb(c, sem):
        pltpu.make_async_copy(kb_v.at[c], kb_v.at[c], sem).wait()
        pltpu.make_async_copy(vb_v.at[c], vb_v.at[c], sem).wait()

    def cp_out_a():
        return pltpu.make_async_copy(outa_v, out_h.at[:, pl.ds(0, D)], sem_out.at[0])

    def cp_out_b(i):
        n0 = sum(OUTC[:i])
        return pltpu.make_async_copy(outb_v.at[:, pl.ds(n0, OUTC[i])],
                                     out_h.at[:, pl.ds(D + n0, OUTC[i])], sem_out.at[0])

    def qproj(s, br, heads, slot=0):
        h0, h1 = heads[0], heads[-1] + 1
        q = _dot(x_v[br], wq_v[s, :, h0 * DH:h1 * DH])
        for h in heads:
            q_v[slot, h] = _pack(q[:, (h - h0) * DH:(h - h0 + 1) * DH])

    def oproj(s, br, n0, n1, first=False, slot=0):
        y = _dot(_unpack(o_v[slot]), wo_v[s, :, n0:n1])
        if not first:
            y = acc_v[br, :, n0:n1] + y
        acc_v[br, :, n0:n1] = y

    lane_grp = lax.broadcasted_iota(jnp.int32, (SK, 128), 1) // SK
    HQ = SQ // 2

    def store_o(slot, b, o4):
        o4 = _pack(o4)
        for h in range(HG):
            o_v[slot, b * HQ:(b + 1) * HQ, h * DH:(h + 1) * DH] = o4[h * HQ:(h + 1) * HQ]

    def qk_gqa(s, bs, slot=0):
        g = s // 2
        for b in bs:
            q4 = jnp.concatenate([q_v[slot, h, b * HQ:(b + 1) * HQ, :] for h in range(HG)], axis=0)
            st = _dot_nt(ka_v[b, g], _unpack(q4))
            pt_v[slot, b // 4, (b % 4) * SK:(b % 4 + 1) * SK, :] = _softmax_t(st)

    def pv_gqa(s, ps=0, oslot=None):
        slot = ps if oslot is None else oslot
        g = s // 2
        z = jnp.zeros((SK, DH), BF16)
        for jb in range(B // 4):
            t = pt_v[ps, jb].T.astype(BF16)
            for j in range(4):
                b = jb * 4 + j
                vp = jnp.concatenate([va_v[b, g] if jj == j else z for jj in range(4)], axis=0)
                store_o(slot, b, _dot(t, vp))

    def qk_mha(s, jbs):
        c = s - NS
        for jb in jbs:
            for h in range(HG):
                kst = jnp.concatenate([kb_v[c, jb * 4 + j, h] for j in range(4)], axis=0)
                st = _dot_nt(kst, _unpack(q_v[0, h, jb * 64:(jb + 1) * 64, :]))
                d = st[0:SK]
                for j in range(1, 4):
                    d = jnp.where(lane_grp == j, st[j * SK:(j + 1) * SK], d)
                pt_v[0, jb, h * SK:(h + 1) * SK, :] = _softmax_t(d)

    lane_grp_h = lax.broadcasted_iota(jnp.int32, (HQ, 128), 1) // SK

    def pv_mha(s, oslot=0):
        c = s - NS
        for jb in range(B // 4):
            t = _pack(pt_v[0, jb].T)
            for j in range(4):
                b = jb * 4 + j
                tj = t[j * HQ:(j + 1) * HQ]
                lhs = jnp.concatenate(
                    [jnp.where(lane_grp_h == h, tj, jnp.uint32(0)) for h in range(HG)], axis=0)
                v4 = vb_v[c, b].reshape(HG * SK, DH)
                store_o(oslot, b, _dot(_unpack(lhs), v4))

    for i in range(len(KP)):
        for c in cp_piece(i):
            c.start()
    for c in cp_kva(0, sem_s.at[0]):
        c.start()
    cp_wq(2, sem_s.at[0]).start()
    cp_wo(0, sem_s.at[1]).start()
    for c in cp_kva(1, sem_s.at[1]):
        c.start()
    for s in range(2, NS):
        if s + 1 == NS:
            cp_xb(sem_s.at[s]).start()
        cp_wq(s + 1, sem_s.at[s]).start()
        cp_wo(s - 1, sem_s.at[s]).start()
    for s in range(NS, 2 * NS):
        for c in cp_kvb(s - NS, sem_s.at[s]):
            c.start()
        if s + 1 < 2 * NS:
            cp_wq(s + 1, sem_s.at[s]).start()
        cp_wo(s - 1, sem_s.at[s]).start()
    cp_wo(2 * NS - 1, sem_s.at[2 * NS - 1]).start()

    acc_v[1] = jnp.zeros((M, D), F32)

    for i in range(len(KP)):
        for c in cp_piece(i):
            c.wait()
        k0 = sum(KP[:i])
        xk = x_v[0, :, k0:k0 + KP[i]]
        for c in range(2):
            y = _dot(xk, wq_v[c, k0:k0 + KP[i], :])
            if i > 0:
                y = y + acc_v[0, :, c * CW:(c + 1) * CW]
            if i + 1 < len(KP):
                acc_v[0, :, c * CW:(c + 1) * CW] = y
            else:
                for h in range(HG):
                    q_v[1 + c, h] = _pack(y[:, h * DH:(h + 1) * DH])

    for c in cp_kva(0, sem_s.at[0]):
        c.wait()
    wait_wq(2, sem_s.at[0])
    qproj(2, 0, [0])
    qk_gqa(0, range(0, 8), 1)
    qproj(2, 0, [1])
    qk_gqa(0, range(8, 16), 1)
    qproj(2, 0, [2])
    qk_gqa(1, range(0, 8), 2)
    qproj(2, 0, [3])
    qk_gqa(1, range(8, 16), 2)
    pv_gqa(0, 1)
    wait_wo(0, sem_s.at[1])
    for c in cp_kva(1, sem_s.at[1]):
        c.wait()
    oproj(0, 0, 0, D, first=True, slot=1)
    pv_gqa(1, 2, oslot=0)

    def body_a(s, carry):
        @pl.when(s == NS - 1)
        def _():
            cp_xb(sem_s.at[s]).wait()
        wait_wq(s + 1, sem_s.at[s])
        wait_wo(s - 1, sem_s.at[s])
        for i in range(4):
            oproj(s - 1, 0, i * 128, (i + 1) * 128)
            qk_gqa(s, range(4 * i, 4 * i + 4))
        oproj(s - 1, 0, 512, D)
        pv_gqa(s)
        qproj(s + 1, (s + 1) // NS, [0, 1, 2, 3])
        return carry

    lax.fori_loop(2, NS, body_a, 0)

    def body_b(s, carry):
        wait_wq(s + 1, sem_s.at[s])
        wait_wo(s - 1, sem_s.at[s])
        wait_kvb(s - NS, sem_s.at[s])
        br = (s - 1) // NS
        for i in range(4):
            oproj(s - 1, br, i * 128, (i + 1) * 128)
            qk_mha(s, [i])
        oproj(s - 1, br, 512, D)
        pv_mha(s)
        r = pl.ds(pl.multiple_of(jnp.minimum((s - NS) * CONV, M - CONV), 16), CONV)
        outa_v[r, :] = acc_v[0, r, :].astype(BF16)
        qproj(s + 1, 1, [0, 1, 2, 3])
        return carry

    lax.fori_loop(NS, 2 * NS - 1, body_b, 0)

    s = 2 * NS - 1
    cp_out_a().start()
    wait_wo(s - 1, sem_s.at[s])
    wait_wo(s, sem_s.at[s])
    wait_kvb(s - NS, sem_s.at[s])
    for i in range(4):
        oproj(s - 1, 1, i * 128, (i + 1) * 128)
        qk_mha(s, [i])
    oproj(s - 1, 1, 512, 768)
    pv_mha(s, oslot=1)
    oproj(s - 1, 1, 768, D)
    for i in range(len(OUTC)):
        n0 = sum(OUTC[:i])
        nn = slice(n0, n0 + OUTC[i])
        outb_v[:, nn] = (acc_v[1, :, nn] + _dot(_unpack(o_v[1]), wo_v[s, :, nn])).astype(BF16)
        cp_out_b(i).start()
    cp_out_a().wait()
    for i in range(len(OUTC)):
        cp_out_b(i).wait()


NSEM = len(KP) + 2 * NS + 1


@jax.jit
def pallas_concat_heads__gqa_block_cached__mha_block_cached__near_ridge_kernel(A_x, A_k_cache, A_v_cache, A_wq, A_wo, B_x, B_k_cache, B_v_cache, B_wq, B_wo):
    any_spec = pl.BlockSpec(memory_space=pl.ANY)
    out = pl.pallas_call(
        kernel,
        out_shape=jax.ShapeDtypeStruct((M, 2 * D), BF16),
        in_specs=[any_spec] * 10,
        out_specs=any_spec,
        scratch_shapes=[
            pltpu.VMEM((2, M, D), BF16),
            pltpu.VMEM((2 * NS, D, CW), BF16),
            pltpu.VMEM((2 * NS, CW, WOP), BF16),
            pltpu.VMEM((B, HKV, SK, DH), BF16),
            pltpu.VMEM((B, HKV, SK, DH), BF16),
            pltpu.VMEM((NS, B, HG, SK, DH), BF16),
            pltpu.VMEM((NS, B, HG, SK, DH), BF16),
            pltpu.VMEM((3, HG, M // 2, DH), U32),
            pltpu.VMEM((3, B // 4, 128, 128), F32),
            pltpu.VMEM((2, M // 2, CW), U32),
            pltpu.VMEM((2, M, D), F32),
            pltpu.VMEM((M, D), BF16),
            pltpu.VMEM((M, D), BF16),
            pltpu.SemaphoreType.DMA((NSEM,)),
        ],
        compiler_params=pltpu.CompilerParams(vmem_limit_bytes=100 * 1024 * 1024),
    )(A_x.reshape(M, D), A_k_cache, A_v_cache, A_wq, A_wo,
      B_x.reshape(M, D), B_k_cache, B_v_cache, B_wq, B_wo)
    return out.reshape(B, SQ, 2 * D)
```

```python
import functools
import math
import jax
import jax.numpy as jnp
from jax import lax
import jax.experimental.pallas as pl
import jax.experimental.pallas.tpu as pltpu

B, SQ, D = 16, 32, 1024
H, DH, SK = 32, 128, 32
HKV = 4
M = B * SQ
HG = 4
NS = H // HG
CW = HG * DH
NJB = B // 4
HQ = SQ // 2
SCALE = DH ** -0.5
EXP2_SCALE = SCALE * math.log2(math.e)
F32 = jnp.float32
BF16 = jnp.bfloat16
U32 = jnp.uint32
PB = (((0, 0, 1), (1, 0, 1)), ((0, 1, 1), (1, 1, 1)), ((0, 2, 2), (1, 2, 1)), ((0, 4, 2), (1, 3, 2)), ((0, 6, 2), (1, 5, 1), (1, 6, 1), (1, 7, 1)))
PX = ((0, 1), (1, 1), (2, 2), (4, 2), (6, 2))
OUTC = (256, 256, 256, 128, 128)
OUTR = (0, 256, 384, 448, 512)
WOP = D + 128
UB = 2

_NT = (((1,), (1,)), ((), ()))


def _dot(a, b):
    return jnp.dot(a, b, preferred_element_type=F32)


def _dot_nt(a, b):
    return lax.dot_general(a, b, _NT, preferred_element_type=F32)


def _pack(x):
    return pltpu.bitcast(x.astype(BF16), U32)


def _unpack(x):
    return pltpu.bitcast(x, BF16)


def _softmax_t(st):
    m = jnp.max(st, axis=0, keepdims=True)
    e = jnp.exp2((st - m) * EXP2_SCALE)
    l = jnp.sum(e, axis=0, keepdims=True)
    r = pl.reciprocal(l, approx=True)
    r = r * (2.0 - l * r)
    return e * r


def kernel(xa_h, ka_h, va_h, wqa_h, woa_h, xb_h, kb_h, vb_h, wqb_h, wob_h, out_h,
           x_v, wq_v, wo_v, ka_v, va_v, kb_v, vb_v, q_v, t_v, o_v, acc_v, outa_v, outb_v, sems):
    off = [0]

    def sem_block(n):
        r = sems.at[pl.ds(off[0], n)]
        off[0] += n
        return r

    sem_p = sem_block(len(PB))
    sem_a = sem_block(NS)
    sem_b = sem_block(NS // UB + 2)
    sem_out = sem_block(1)

    def cp_piece(i):
        sem = sem_p.at[i]
        k0, nk = PX[i]
        kk = pl.ds(k0 * 128, nk * 128)
        cps = [pltpu.make_async_copy(xa_h.at[:, kk], x_v.at[0, :, kk], sem)]
        for c, k0, nk in PB[i]:
            kk = pl.ds(k0 * 128, nk * 128)
            cps.append(pltpu.make_async_copy(wqa_h.at[kk, pl.ds(c * CW, CW)], wq_v.at[c, kk, :], sem))
        if i + 1 == len(PB):
            gs = pl.ds(0, 1)
            cps.append(pltpu.make_async_copy(ka_h.at[:, gs], ka_v.at[:, gs], sem))
        return cps

    def cp_wq(s, sem):
        src = (wqa_h, wqb_h)[s // NS]
        c = s % NS
        return pltpu.make_async_copy(src.at[:, pl.ds(c * CW, CW)], wq_v.at[s], sem)

    def cp_wo(s, sem):
        src = (woa_h, wob_h)[s // NS]
        c = s % NS
        return pltpu.make_async_copy(src.at[pl.ds(c * CW, CW), :], wo_v.at[s, :, pl.ds(0, D)], sem)

    def cp_va0(sem):
        gs = pl.ds(0, 1)
        return pltpu.make_async_copy(va_h.at[:, gs], va_v.at[:, gs], sem)

    def cp_kva_rest(sem):
        gs = pl.ds(1, HKV - 1)
        return [
            pltpu.make_async_copy(ka_h.at[:, gs], ka_v.at[:, gs], sem),
            pltpu.make_async_copy(va_h.at[:, gs], va_v.at[:, gs], sem),
        ]

    def cp_xb(sem):
        return pltpu.make_async_copy(xb_h, x_v.at[1], sem)

    def cp_kb(s, sem):
        c = s - NS
        return [pltpu.make_async_copy(kb_h.at[:, pl.ds(c * HG, HG)], kb_v.at[c], sem)]

    def cp_vb(s, sem):
        if s == NS - 1:
            return [pltpu.make_async_copy(va_h.at[pl.ds(0, 4), pl.ds(HKV - 1, 1)],
                                          vb_v.at[0, pl.ds(0, 4), pl.ds(h, 1)], sem)
                    for h in range(HG)]
        c = s - NS
        return [pltpu.make_async_copy(vb_h.at[:, pl.ds(c * HG, HG)], vb_v.at[c + 1], sem)]

    def wait_ref(r, sem):
        pltpu.make_async_copy(r, r, sem).wait()

    def wait_wq(s, sem):
        wait_ref(wq_v.at[s], sem)

    def wait_wo(s, sem):
        wait_ref(wo_v.at[s, :, pl.ds(0, D)], sem)

    def wait_kb(s, sem):
        wait_ref(kb_v.at[s - NS], sem)

    def wait_vb(s, sem):
        wait_ref(vb_v.at[s - (NS - 1)], sem)

    def cp_out_a():
        return pltpu.make_async_copy(outa_v, out_h.at[:, pl.ds(0, D)], sem_out.at[0])

    def cp_out_b(i, r0, r1):
        n0 = sum(OUTC[:i])
        rr = pl.ds(r0, r1 - r0)
        return pltpu.make_async_copy(outb_v.at[rr, pl.ds(n0, OUTC[i])],
                                     out_h.at[rr, pl.ds(D + n0, OUTC[i])], sem_out.at[0])

    def store_q(slot, q):
        for h in range(HG):
            q_v[slot, h] = _pack(q[:, h * DH:(h + 1) * DH])

    def qproj(s, br):
        store_q(0, _dot(x_v[br], wq_v[s]))

    def oproj(s, br, n0, n1, first=False):
        y = _dot(_unpack(o_v[...]), wo_v[s, :, n0:n1])
        if not first:
            y = acc_v[br, :, n0:n1] + y
        acc_v[br, :, n0:n1] = y

    lane_grp = lax.broadcasted_iota(jnp.int32, (SK, 128), 1) // SK
    lane_grp_h = lax.broadcasted_iota(jnp.int32, (HQ, 128), 1) // SK
    zkv = jnp.zeros((SK, DH), BF16)

    def load_q4(slot, b):
        return _unpack(jnp.concatenate(
            [q_v[slot, h, b * HQ:(b + 1) * HQ, :] for h in range(HG)], axis=0))

    def qk_gqa(s, jb, slot=0):
        g = s >> 1
        pts = []
        for j in range(4):
            b = jb * 4 + j
            st = _dot_nt(ka_v[b, g], load_q4(slot, b))
            pts.append(_softmax_t(st))
        t_v[jb] = _pack(jnp.concatenate(pts, axis=0).T)

    def qk_mha(s, jb):
        c = s - NS
        pts = []
        for j in range(4):
            b = jb * 4 + j
            st = _dot_nt(kb_v[c, b].reshape(HG * SK, DH), load_q4(0, b))
            d = st[0:SK]
            for h in range(1, HG):
                d = jnp.where(lane_grp == h, st[h * SK:(h + 1) * SK], d)
            pts.append(_softmax_t(d))
        t_v[jb] = _pack(jnp.concatenate(pts, axis=0).T)

    def pv_gqa(s, jbs):
        g = s >> 1
        for jb in jbs:
            for j in range(4):
                b = jb * 4 + j
                vp = jnp.concatenate([va_v[b, g] if jj == j else zkv for jj in range(4)], axis=0)
                o4 = _pack(_dot(_unpack(t_v[jb]), vp))
                for h in range(HG):
                    o_v[b * HQ:(b + 1) * HQ, h * DH:(h + 1) * DH] = o4[h * HQ:(h + 1) * HQ]

    def pv_masked(vget, jb, j0=0):
        for h in range(HG):
            th = t_v[jb, h * HQ:(h + 1) * HQ, :]
            lhs = jnp.concatenate(
                [jnp.where(lane_grp_h == j, th, jnp.uint32(0)) for j in range(j0, 4)], axis=0)
            vst = jnp.concatenate([vget(jb * 4 + j, h) for j in range(4)], axis=0)
            o_v[(jb * 4 + j0) * HQ:(jb + 1) * 4 * HQ, h * DH:(h + 1) * DH] = _pack(_dot(_unpack(lhs), vst))

    def pv_first(vget):
        for h in range(HG):
            vp = jnp.concatenate([vget(0, h), zkv, zkv, zkv], axis=0)
            o_v[0:HQ, h * DH:(h + 1) * DH] = _pack(_dot(_unpack(t_v[0, h * HQ:(h + 1) * HQ, :]), vp))
        pv_masked(vget, 0, 1)

    def vget_a(s):
        return lambda b, h: va_v[b, s >> 1]

    def vget_b(s):
        return lambda b, h: vb_v[s - (NS - 1), b, h]

    def pv_mha(s, jbs):
        for jb in jbs:
            pv_masked(vget_b(s), jb)

    def oproj_qk(so, br, qk, first=False, post=None):
        for k in range(NJB):
            oproj(so, br, k * 128, (k + 1) * 128, first)
            qk((k + 1) % NJB)
        if post is None:
            oproj(so, br, NJB * 128, D, first)
        else:
            for k in range(4):
                post(k)
                oproj(so, br, (NJB + k) * 128, (NJB + k + 1) * 128, first)

    for i in range(len(PB)):
        for c in cp_piece(i):
            c.start()
    cp_va0(sem_a.at[1]).start()
    cp_wo(0, sem_a.at[1]).start()
    for c in cp_kva_rest(sem_a.at[0]):
        c.start()
    for s in range(2, NS):
        cp_wq(s, sem_a.at[s]).start()
        cp_wo(s - 1, sem_a.at[s]).start()
    for c in cp_vb(NS - 1, sem_b.at[NS // UB + 1]) + [cp_xb(sem_b.at[NS // UB + 1])]:
        c.start()
    for s in range(NS, 2 * NS):
        sem = sem_b.at[(s - NS) // UB]
        for c in [cp_wq(s, sem), cp_wo(s - 1, sem)] + cp_kb(s, sem) + cp_vb(s, sem):
            c.start()
    cp_wo(2 * NS - 1, sem_b.at[NS // UB]).start()

    acc_v[1] = jnp.zeros((M, D), F32)

    for i in range(len(PB)):
        for c in cp_piece(i):
            c.wait()
        for r, (c, k0, nk) in enumerate(PB[i]):
            kk = slice(k0 * 128, (k0 + nk) * 128)
            y = _dot(x_v[0, :, kk], wq_v[c, kk, :])
            if k0 > 0:
                y = y + acc_v[0, :, c * CW:(c + 1) * CW]
            if k0 + nk < D // 128:
                acc_v[0, :, c * CW:(c + 1) * CW] = y
            else:
                store_q(1 - c, y)
            if i + 1 == len(PB) and r in (1, 2):
                qk_gqa(0, 2 * (r - 1), 1)
                qk_gqa(0, 2 * (r - 1) + 1, 1)

    rest = range(1, NJB)
    cp_va0(sem_a.at[1]).wait()
    wait_wo(0, sem_a.at[1])
    pv_first(vget_a(0))
    pv_gqa(0, rest)
    oproj_qk(0, 0, lambda jb: qk_gqa(1, jb), first=True)
    pv_gqa(1, rest)
    for c in cp_kva_rest(sem_a.at[0]):
        c.wait()

    def body_a(s, carry):
        wait_wq(s, sem_a.at[s])
        wait_wo(s - 1, sem_a.at[s])
        pv_first(vget_a(s - 1))
        qproj(s, 0)
        oproj_qk(s - 1, 0, lambda jb: qk_gqa(s, jb))
        pv_gqa(s, rest)
        return carry

    lax.fori_loop(2, NS, body_a, 0)
    for c in cp_vb(NS - 1, sem_b.at[NS // UB + 1]) + [cp_xb(sem_b.at[NS // UB + 1])]:
        c.wait()

    conv = M // (NS // UB)

    def body_b(i, carry):
        s0 = NS + i * UB
        sem = sem_b.at[i]
        for u in range(UB):
            wait_wq(s0 + u, sem)
            wait_wo(s0 + u - 1, sem)
            wait_kb(s0 + u, sem)
            wait_vb(s0 + u, sem)
        pv_first(vget_b(s0 - 1))
        for u in range(UB):
            s = s0 + u
            qproj(s, 1)
            def post(k):
                cu = conv // (UB // 2) // 4
                r = pl.ds(pl.multiple_of(i * conv + ((u // 2) * 4 + k) * cu, cu), cu)
                outa_v[r, :] = acc_v[0, r, :].astype(BF16)
            oproj_qk(s - 1, jnp.minimum(i, 1) if u == 0 else 1, lambda jb: qk_mha(s, jb),
                     post=post if u % 2 == 1 else None)
            pv_mha(s, rest if u + 1 == UB else (1, 2, 3, 0))
        return carry

    lax.fori_loop(0, NS // UB, body_b, 0)

    s = 2 * NS - 1
    outs = [cp_out_a()]
    outs[0].start()
    wait_wo(s, sem_b.at[NS // UB])
    pv_first(vget_b(s))
    for i in range(len(OUTC)):
        n0 = sum(OUTC[:i])
        nn = slice(n0, n0 + OUTC[i])
        y = (acc_v[1, :, nn] + _dot(_unpack(o_v[...]), wo_v[s, :, nn])).astype(BF16)
        rows = OUTR if i + 1 == len(OUTC) else (0, M)
        for r0, r1 in zip(rows[:-1], rows[1:]):
            outb_v[r0:r1, nn] = y[r0:r1]
            outs.append(cp_out_b(i, r0, r1))
            outs[-1].start()
    for c in outs:
        c.wait()


NSEM = len(PB) + NS + NS // UB + 2 + 1


@jax.jit
def pallas_concat_heads__gqa_block_cached__mha_block_cached__near_ridge_kernel(A_x, A_k_cache, A_v_cache, A_wq, A_wo, B_x, B_k_cache, B_v_cache, B_wq, B_wo):
    any_spec = pl.BlockSpec(memory_space=pl.ANY)
    out = pl.pallas_call(
        kernel,
        out_shape=jax.ShapeDtypeStruct((M, 2 * D), BF16),
        in_specs=[any_spec] * 10,
        out_specs=any_spec,
        scratch_shapes=[
            pltpu.VMEM((2, M, D), BF16),
            pltpu.VMEM((2 * NS, D, CW), BF16),
            pltpu.VMEM((2 * NS, CW, WOP), BF16),
            pltpu.VMEM((B, HKV, SK, DH), BF16),
            pltpu.VMEM((B, HKV, SK, DH), BF16),
            pltpu.VMEM((NS, B, HG, SK, DH), BF16),
            pltpu.VMEM((NS + 1, B, HG, SK, DH), BF16),
            pltpu.VMEM((2, HG, M // 2, DH), U32),
            pltpu.VMEM((NJB, 64, 128), U32),
            pltpu.VMEM((M // 2, CW), U32),
            pltpu.VMEM((2, M, D), F32),
            pltpu.VMEM((M, D), BF16),
            pltpu.VMEM((M, D), BF16),
            pltpu.SemaphoreType.DMA((NSEM,)),
        ],
        compiler_params=pltpu.CompilerParams(vmem_limit_bytes=100 * 1024 * 1024,
            disable_semaphore_checks=True, disable_bounds_checks=True),
    )(A_x.reshape(M, D), A_k_cache, A_v_cache, A_wq, A_wo,
      B_x.reshape(M, D), B_k_cache, B_v_cache, B_wq, B_wo)
    return out.reshape(B, SQ, 2 * D)
```

```python
import math

import jax
import jax.numpy as jnp
from jax import lax
import jax.experimental.pallas as pl
import jax.experimental.pallas.tpu as pltpu

B, SQ, D = 16, 32, 1024
H, DH, SK = 32, 128, 32
HKV = 4
M = B * SQ
HG = 4
NS = H // HG
CW = HG * DH
NJB = B // 4
HQ = SQ // 2
UB = 4
NB = NS // UB
WOP = D + 128
SCALE_BF16 = 0.08837890625
LOG2E = math.log2(math.e)
F32 = jnp.float32
BF16 = jnp.bfloat16
U32 = jnp.uint32

PB = (
    ((0, 0, 1), (1, 0, 1)),
    ((0, 1, 1), (1, 1, 1)),
    ((0, 2, 2), (1, 2, 1)),
    ((0, 4, 2), (1, 3, 2)),
    ((0, 6, 2), (1, 5, 1), (1, 6, 1), (1, 7, 1)),
)
PX = ((0, 1), (1, 1), (2, 2), (4, 2), (6, 2))
OUTC = (256, 256, 256, 128, 128)
OUTR = (0, 256, 384, 448, 512)

SEM_P = 0
SEM_A = SEM_P + len(PB)
SEM_B = SEM_A + NS
SEM_LAST = SEM_B + NB
SEM_XB = SEM_LAST + 1
SEM_OUT = SEM_XB + 1
NSEM = SEM_OUT + 1


def _dot(a, b):
    return jnp.dot(a, b, preferred_element_type=F32)


def _dot_nt(a, b):
    return lax.dot_general(a, b, (((1,), (1,)), ((), ())), preferred_element_type=F32)


def _pack(x):
    return pltpu.bitcast(x.astype(BF16), U32)


def _unpack(x):
    return pltpu.bitcast(x, BF16)


def _softmax_t(st):
    st = (st.astype(BF16).astype(F32) * SCALE_BF16).astype(BF16).astype(F32)
    m = jnp.max(st, axis=0, keepdims=True)
    e = jnp.exp2((st - m) * LOG2E)
    l = jnp.sum(e, axis=0, keepdims=True)
    r = pl.reciprocal(l, approx=True)
    r = r * (2.0 - l * r)
    return e * r


def _kernel(xa_h, ka_h, va_h, wqa_h, woa_h, xb_h, kb_h, vb_h, wqb_h, wob_h, out_h,
            x_v, wq_v, wo_v, ka_v, va_v, kb_v, vb_v, q_v, t_v, o_v, acc_v, outa_v, outb_v, sems):
    copy = pltpu.make_async_copy

    def cp_block(i):
        sem = sems.at[SEM_P + i]
        kk = pl.ds(PX[i][0] * 128, PX[i][1] * 128)
        cps = [copy(xa_h.at[:, kk], x_v.at[0, :, kk], sem)]
        for c, k0, nk in PB[i]:
            kk = pl.ds(k0 * 128, nk * 128)
            cps.append(copy(wqa_h.at[kk, pl.ds(c * CW, CW)], wq_v.at[c, kk, :], sem))
        if i + 1 == len(PB):
            cps.append(copy(ka_h.at[:, pl.ds(0, 1)], ka_v.at[:, pl.ds(0, 1)], sem))
        return cps

    def cp_wq(s, sem):
        src = (wqa_h, wqb_h)[s // NS]
        return copy(src.at[:, pl.ds((s % NS) * CW, CW)], wq_v.at[s], sem)

    def cp_wo(s, sem):
        src = (woa_h, wob_h)[s // NS]
        return copy(src.at[pl.ds((s % NS) * CW, CW), :], wo_v.at[s, :, pl.ds(0, D)], sem)

    def cp_step1():
        sem = sems.at[SEM_A + 1]
        return [copy(va_h.at[:, pl.ds(0, 1)], va_v.at[:, pl.ds(0, 1)], sem), cp_wo(0, sem)]

    def cp_kva_rest():
        sem, gs = sems.at[SEM_A], pl.ds(1, HKV - 1)
        return [copy(ka_h.at[:, gs], ka_v.at[:, gs], sem), copy(va_h.at[:, gs], va_v.at[:, gs], sem)]

    def cp_xb():
        sem = sems.at[SEM_XB]
        cps = [copy(va_h.at[pl.ds(0, 4), pl.ds(HKV - 1, 1)], vb_v.at[0, pl.ds(0, 4), pl.ds(h, 1)], sem)
               for h in range(HG)]
        return cps + [copy(xb_h, x_v.at[1], sem)]

    def cp_kvb(s, sem):
        hs = pl.ds((s - NS) * HG, HG)
        return [copy(kb_h.at[:, hs], kb_v.at[s - NS], sem), copy(vb_h.at[:, hs], vb_v.at[s - NS + 1], sem)]

    def wait_into(ref, sem):
        copy(ref, ref, sem).wait()

    def wait_w(s, sem):
        wait_into(wq_v.at[s], sem)
        wait_into(wo_v.at[s - 1, :, pl.ds(0, D)], sem)

    lane_grp = lax.broadcasted_iota(jnp.int32, (SK, 128), 1) // SK
    lane_grp_h = lax.broadcasted_iota(jnp.int32, (HQ, 128), 1) // SK
    zkv = jnp.zeros((SK, DH), BF16)

    def qproj(s, br):
        x = x_v[br]
        for h in range(HG):
            q_v[0, :, h * DH:(h + 1) * DH] = _pack(_dot(x, wq_v[s, :, h * DH:(h + 1) * DH]))

    def oproj(s, br, n0, n1, first=False, r0=0, r1=M):
        y = _dot(_unpack(o_v[r0 // 2:r1 // 2, :]), wo_v[s, :, n0:n1])
        if not first:
            y = acc_v[br, r0:r1, n0:n1] + y
        acc_v[br, r0:r1, n0:n1] = y

    def load_q4(slot, b):
        return _unpack(jnp.concatenate(
            [q_v[slot, b * HQ:(b + 1) * HQ, h * DH:(h + 1) * DH] for h in range(HG)], axis=0))

    def store_t(jb, pts):
        t_v[jb] = pltpu.bitcast(jnp.concatenate(pts, axis=0).astype(BF16).T, U32)

    def qk_gqa(s, jb, slot=0):
        pts = []
        for j in range(4):
            b = jb * 4 + j
            pts.append(_softmax_t(_dot_nt(ka_v[b, s >> 1], load_q4(slot, b))))
        store_t(jb, pts)

    def qk_mha_half(s, jb, half):
        pts = []
        for j in range(2 * half, 2 * half + 2):
            b = jb * 4 + j
            q4 = load_q4(0, b)
            d = None
            for hh in range(2):
                st = _dot_nt(kb_v[s - NS, b, 2 * hh:2 * hh + 2].reshape(2 * SK, DH), q4)
                for h2 in range(2):
                    blk = st[h2 * SK:(h2 + 1) * SK]
                    d = blk if d is None else jnp.where(lane_grp == 2 * hh + h2, blk, d)
            pts.append(_softmax_t(d))
        return pts

    def pv(vget, jb, j0=0):
        for h in range(HG):
            th = t_v[jb, h * HQ:(h + 1) * HQ, :]
            lhs = jnp.concatenate(
                [jnp.where(lane_grp_h == j, th, jnp.uint32(0)) for j in range(j0, 4)], axis=0)
            vst = jnp.concatenate([vget(jb * 4 + j, h) for j in range(4)], axis=0)
            o_v[(jb * 4 + j0) * HQ:(jb + 1) * 4 * HQ, h * DH:(h + 1) * DH] = _pack(_dot(_unpack(lhs), vst))

    def pv_first(vget):
        for h in range(HG):
            vp = jnp.concatenate([vget(0, h), zkv, zkv, zkv], axis=0)
            o_v[0:HQ, h * DH:(h + 1) * DH] = _pack(_dot(_unpack(t_v[0, h * HQ:(h + 1) * HQ, :]), vp))
        pv(vget, 0, 1)

    def vget_a(s):
        return lambda b, h: va_v[b, s >> 1]

    def vget_b(s):
        return lambda b, h: vb_v[s - (NS - 1), b, h]

    def oproj_qk_gqa(s, first=False):
        for k in range(NJB):
            oproj(s - 1, 0, k * 128, (k + 1) * 128, first)
            qk_gqa(s, (k + 1) % NJB)
        oproj(s - 1, 0, NJB * 128, D, first)

    def oproj_qk_mha(s, br, post=None):
        for k in range(NJB):
            jb = (k + 1) % NJB
            oproj(s - 1, br, k * 128, (k + 1) * 128, r0=0, r1=M // 2)
            pts = qk_mha_half(s, jb, 0)
            oproj(s - 1, br, k * 128, (k + 1) * 128, r0=M // 2, r1=M)
            pts += qk_mha_half(s, jb, 1)
            store_t(jb, pts)
        if post is None:
            oproj(s - 1, br, NJB * 128, D)
        else:
            for k in range(4):
                post(k)
                oproj(s - 1, br, (NJB + k) * 128, (NJB + k + 1) * 128)

    starts = []
    for i in range(len(PB)):
        starts += cp_block(i)
    starts += cp_step1() + cp_kva_rest()
    for s in range(2, NS):
        starts += [cp_wq(s, sems.at[SEM_A + s]), cp_wo(s - 1, sems.at[SEM_A + s])]
    starts += cp_xb()
    for s in range(NS, 2 * NS):
        sem = sems.at[SEM_B + (s - NS) // UB]
        starts += [cp_wq(s, sem), cp_wo(s - 1, sem)] + cp_kvb(s, sem)
    starts.append(cp_wo(2 * NS - 1, sems.at[SEM_LAST]))
    for c in starts:
        c.start()

    def zero_acc(i, carry):
        acc_v[1, pl.ds(pl.multiple_of(i * 32, 32), 32), :] = jnp.zeros((32, D), F32)
        return carry

    lax.fori_loop(0, M // 32, zero_acc, 0)

    for i in range(len(PB)):
        for c in cp_block(i):
            c.wait()
        for r, (c, k0, nk) in enumerate(PB[i]):
            kk = slice(k0 * 128, (k0 + nk) * 128)
            y = _dot(x_v[0, :, kk], wq_v[c, kk, :])
            if k0 > 0:
                y = y + acc_v[0, :, c * CW:(c + 1) * CW]
            if k0 + nk < D // 128:
                acc_v[0, :, c * CW:(c + 1) * CW] = y
            else:
                q_v[1 - c] = _pack(y)
            if i + 1 == len(PB) and r in (1, 2):
                qk_gqa(0, 2 * (r - 1), 1)
                qk_gqa(0, 2 * (r - 1) + 1, 1)

    rest = range(1, NJB)
    for c in cp_step1():
        c.wait()
    pv_first(vget_a(0))
    for jb in rest:
        pv(vget_a(0), jb)
    oproj_qk_gqa(1, first=True)
    for jb in rest:
        pv(vget_a(1), jb)
    for c in cp_kva_rest():
        c.wait()

    def body_a(s, carry):
        wait_w(s, sems.at[SEM_A + s])
        pv_first(vget_a(s - 1))
        qproj(s, 0)
        oproj_qk_gqa(s)
        for jb in rest:
            pv(vget_a(s), jb)
        return carry

    lax.fori_loop(2, NS, body_a, 0)
    for c in cp_xb():
        c.wait()

    cu = M // (NB * (UB // 2) * 4)

    def body_b(i, carry):
        s0 = NS + i * UB
        sem = sems.at[SEM_B + i]
        for u in range(UB):
            wait_w(s0 + u, sem)
            wait_into(kb_v.at[s0 + u - NS], sem)
            wait_into(vb_v.at[s0 + u - NS + 1], sem)
        pv_first(vget_b(s0 - 1))
        for u in range(UB):
            s = s0 + u

            def post(k, u=u):
                r = pl.ds(pl.multiple_of(((i * (UB // 2) + u // 2) * 4 + k) * cu, cu), cu)
                outa_v[r, :] = acc_v[0, r, :].astype(BF16)

            qproj(s, 1)
            oproj_qk_mha(s, jnp.minimum(i, 1) if u == 0 else 1, post=post if u % 2 == 1 else None)
            for jb in (rest if u + 1 == UB else (1, 2, 3, 0)):
                pv(vget_b(s), jb)
        return carry

    lax.fori_loop(0, NB, body_b, 0)

    s = 2 * NS - 1
    sem = sems.at[SEM_OUT]
    outs = [copy(outa_v, out_h.at[:, pl.ds(0, D)], sem)]
    outs[0].start()
    cp_wo(s, sems.at[SEM_LAST]).wait()
    pv_first(vget_b(s))
    n0 = 0
    for i, nc in enumerate(OUTC):
        nn = slice(n0, n0 + nc)
        y = (acc_v[1, :, nn] + _dot(_unpack(o_v[...]), wo_v[s, :, nn])).astype(BF16)
        rows = OUTR if i + 1 == len(OUTC) else (0, M)
        for r0, r1 in zip(rows[:-1], rows[1:]):
            outb_v[r0:r1, nn] = y[r0:r1]
            rr = pl.ds(r0, r1 - r0)
            outs.append(copy(outb_v.at[rr, pl.ds(n0, nc)], out_h.at[rr, pl.ds(D + n0, nc)], sem))
            outs[-1].start()
        n0 += nc
    for c in outs:
        c.wait()


@jax.jit
def pallas_concat_heads__gqa_block_cached__mha_block_cached__near_ridge_kernel(
    A_x: jax.Array,
    A_k_cache: jax.Array,
    A_v_cache: jax.Array,
    A_wq: jax.Array,
    A_wo: jax.Array,
    B_x: jax.Array,
    B_k_cache: jax.Array,
    B_v_cache: jax.Array,
    B_wq: jax.Array,
    B_wo: jax.Array,
):
    any_spec = pl.BlockSpec(memory_space=pl.ANY)
    out = pl.pallas_call(
        _kernel,
        out_shape=jax.ShapeDtypeStruct((M, 2 * D), BF16),
        in_specs=[any_spec] * 10,
        out_specs=any_spec,
        scratch_shapes=[
            pltpu.VMEM((2, M, D), BF16),
            pltpu.VMEM((2 * NS, D, CW), BF16),
            pltpu.VMEM((2 * NS, CW, WOP), BF16),
            pltpu.VMEM((B, HKV, SK, DH), BF16),
            pltpu.VMEM((B, HKV, SK, DH), BF16),
            pltpu.VMEM((NS, B, HG, SK, DH), BF16),
            pltpu.VMEM((NS + 1, B, HG, SK, DH), BF16),
            pltpu.VMEM((2, M // 2, CW), U32),
            pltpu.VMEM((NJB, 64, 128), U32),
            pltpu.VMEM((M // 2, CW), U32),
            pltpu.VMEM((2, M, D), F32),
            pltpu.VMEM((M, D), BF16),
            pltpu.VMEM((M, D), BF16),
            pltpu.SemaphoreType.DMA((NSEM,)),
        ],
        compiler_params=pltpu.CompilerParams(
            vmem_limit_bytes=100 * 1024 * 1024,
            disable_semaphore_checks=True,
        ),
    )(A_x.reshape(M, D), A_k_cache, A_v_cache, A_wq, A_wo,
      B_x.reshape(M, D), B_k_cache, B_v_cache, B_wq, B_wo)
    return out.reshape(B, SQ, 2 * D)
```
